```python
import os as _os
_os.environ.setdefault("JAX_PLATFORMS", "cpu")
import jax
import jax.numpy as jnp

def _softmax(x, axis=-1):
    return jax.nn.softmax(x, axis=axis)
def _gelu(x):
    return jax.nn.gelu(x, approximate=True)
def _silu(x):
    return jax.nn.silu(x)
def _sigmoid(x):
    return jax.nn.sigmoid(x)
def _layernorm(x, axis=-1, eps=1e-5):
    m = jnp.mean(x, axis=axis, keepdims=True)
    v = jnp.var(x, axis=axis, keepdims=True)
    return (x - m) / jnp.sqrt(v + eps)
def _scatter_add(tgt, idx, src, axis=0):
    return tgt.at[idx].add(src)
def _segment_sum(src, seg, n):
    return jax.ops.segment_sum(src, seg, n)
class _Rng:
    def __init__(self, key):
        self._k = key
    def _next(self):
        self._k, sub = jax.random.split(self._k)
        return sub
    def normal(self, shape):
        return jax.random.normal(self._next(), shape, dtype=jnp.bfloat16)
    def randint(self, lo, hi, shape):
        return jax.random.randint(self._next(), shape, lo, hi, dtype=jnp.int32)
    def uniform(self, shape, lo=0.0, hi=1.0):
        return jax.random.uniform(self._next(), shape, jnp.bfloat16, lo, hi)
    def permutation(self, n):
        return jax.random.permutation(self._next(), n)


kernel_name = 'interleave_layers__linear_kernel_hedgehog__dense_activation_silu__prompt'

def setup_inputs():
    _rng = _Rng(jax.random.key(int.from_bytes(__import__("os").urandom(4), "little")))
    _w = (lambda a: (lambda t: t.astype(jnp.bfloat16) if jnp.issubdtype(t.dtype, jnp.floating) else t)(jnp.asarray(a)))
    def _A_setup():
        B, S, D, H = 1, 2048, 640, 32
        Dh = D // H
        return {
            "x": _w((lambda *s: _rng.normal(s) * 0.05)(B, S, D)),
            "wqkv": _w((lambda *s: _rng.normal(s) * 0.4)(D, 3 * D)),
            "w_phi": _w((lambda *s: _rng.normal(s) * 0.4)(H, Dh, Dh) * (Dh ** -0.5)),
            "wo": _w((lambda *s: _rng.normal(s) * 0.05)(D, D)),
        }
    _A_in = _A_setup()

    def _B_setup():
        B, S, D, F = 1, 2048, 640, 1728
        return {
            "x": _w((lambda *s: _rng.normal(s) * 0.05)(B, S, D)),
            "w1": _w((lambda *s: _rng.normal(s) * 1.6)(D, F) * (D ** -0.5)),
            "w2": _w((lambda *s: _rng.normal(s) * 1.6)(F, D) * (F ** -0.5)),
        }
    _B_in = _B_setup()

    return {
        "A_x": _A_in["x"],
        "A_wqkv": _A_in["wqkv"],
        "A_w_phi": _A_in["w_phi"],
        "A_wo": _A_in["wo"],
        "B_x": _B_in["x"],
        "B_w1": _B_in["w1"],
        "B_w2": _B_in["w2"],
    }

def reference(A_x, A_wqkv, A_w_phi, A_wo, B_x, B_w1, B_w2):
    def _A_ref(x, wqkv, w_phi, wo):
        B, S, D = x.shape
        H = 32; Dh = D // H
        qkv = (lambda x, *d: x.transpose(*d))((x @ wqkv).reshape(B, S, 3, H, Dh), 2, 0, 3, 1, 4)
        q, k, v = qkv[0], qkv[1], qkv[2]
        pq = jnp.einsum("bhsd,hdf->bhsf", q, w_phi)
        pk = jnp.einsum("bhsd,hdf->bhsf", k, w_phi)
        phi_q = jnp.concatenate([_softmax(pq, axis=-1), _softmax(-pq, axis=-1)], axis=-1)
        phi_k = jnp.concatenate([_softmax(pk, axis=-1), _softmax(-pk, axis=-1)], axis=-1)
        kv = jnp.einsum("bhsf,bhsd->bhfd", phi_k, v)
        z  = jnp.einsum("bhsf->bhf", phi_k)
        num = jnp.einsum("bhqf,bhfd->bhqd", phi_q, kv)
        den = jnp.einsum("bhqf,bhf->bhq", phi_q, z)[..., None] + 1e-6
        o = num / den
        return (lambda x, *d: x.transpose(*d))(o, 0, 2, 1, 3).reshape(B, S, D) @ wo

    def _B_ref(x, w1, w2):
        h = jnp.einsum("bsd,df->bsf", x, w1)
        h = _silu(h)
        out = jnp.einsum("bsf,fd->bsd", h, w2)
        return out

    x = A_x
    x = x + _A_ref(_layernorm(x, axis=-1), A_wqkv, A_w_phi, A_wo)
    x = x + _B_ref(_layernorm(x, axis=-1), B_w1, B_w2)
    x = x + _A_ref(_layernorm(x, axis=-1), A_wqkv, A_w_phi, A_wo)
    x = x + _B_ref(_layernorm(x, axis=-1), B_w1, B_w2)
    return x
```

```python
import functools
import math
import jax
import jax.numpy as jnp
from jax import lax
import jax.experimental.pallas as pl
import jax.experimental.pallas.tpu as pltpu

S, D, H, DH, F = 2048, 640, 32, 20, 1728
SC = 256
NCH = S // SC
NS = 2
STAT_ORDER = "0100112201"
UPD_ORDER = "0101010101"
FLAGS = {"XLA_TPU_EVENLY_DISTRIBUTE_CRITICAL_NODES": True}
LNB = 32
NB2 = 128
LOG2E = 1.4426950408889634
F32, BF16 = jnp.float32, jnp.bfloat16

NT = (((1,), (1,)), ((), ()))
NN = (((1,), (0,)), ((), ()))

CH_PAIRS = [((128 * c) // 80, (128 * c + 127) // 80 + 1) for c in range(5)]


def _dot(a, b, dims):
    return lax.dot_general(a, b, dims, preferred_element_type=F32)


def _iota(shape, dim):
    return lax.broadcasted_iota(jnp.int32, shape, dim)


def _div_small(v, d, vmax):
    out = jnp.zeros_like(v)
    for t in range(d, vmax, d):
        out = out + (v >= t).astype(jnp.int32)
    return out


def _layernorm(x, scale):
    m = jnp.mean(x, axis=-1, keepdims=True)
    xc = x - m
    v = jnp.mean(xc * xc, axis=-1, keepdims=True)
    return (xc * (lax.rsqrt(v + 1e-5) * scale)).astype(BF16)


def _pair_reduce(y, op):
    y = op(y, pltpu.roll(y, 4, 0))
    return op(y, pltpu.roll(y, 2, 0))


def _hedgehog_pair(p):
    ps = [p[8 * i:8 * i + 8] for i in range(5)]
    mx = _pair_reduce(functools.reduce(jnp.maximum, ps), jnp.maximum)
    mn = _pair_reduce(functools.reduce(jnp.minimum, ps), jnp.minimum)
    ep = [jnp.exp2(q - mx) for q in ps]
    em = [jnp.exp2(mn - q) for q in ps]
    rp = 1.0 / _pair_reduce(functools.reduce(jnp.add, ep), jnp.add)
    rm = 1.0 / _pair_reduce(functools.reduce(jnp.add, em), jnp.add)
    return jnp.concatenate([e * rp for e in ep] + [e * rm for e in em], axis=0).astype(BF16)


def _interleave(gens, order):
    gens = list(gens)
    for ch in order:
        next(gens[int(ch)])
    done = object()
    for g in gens:
        assert next(g, done) is done


def kernel(x_hbm, wqkv_hbm, wphi_hbm, wo_hbm, w1_hbm, w2_hbm, out_hbm,
           xres, wqkv, wphi, wo, w1, w2, wqT, wkvT, xn_s, kvacc, kvl,
           h_s, phi_s, vx_s, p_s, x1_s, bd_s, xh_s, sem_x, sem_w, sem_o):
    cx = [pltpu.make_async_copy(x_hbm.at[pl.ds(i * SC, SC)], xres.at[pl.ds(i * SC, SC)], sem_x.at[i])
          for i in range(NCH)]
    cols = [pl.ds(j * D, D) for j in range(3)]
    cw = [pltpu.make_async_copy(a, b, sem_w.at[i]) for i, (a, b) in enumerate(
        [(wphi_hbm, wphi), (wo_hbm, wo), (w1_hbm, w1), (w2_hbm, w2)]
        + [(wqkv_hbm.at[:, c], wqkv.at[:, c]) for c in cols])]
    c_phi, c_wo, c_w1, c_w2, c_wq, c_wk, c_wv = cw
    c_phi.start()
    c_wq.start()
    c_wk.start()

    c_phi.wait()
    rho = _iota((160, 128), 0)
    f_of = (rho - 40 * _div_small(rho, 40, 160)) >> 1
    eT = (f_of == _iota((160, 128), 1)).astype(BF16)[:, :DH]
    rho2 = _iota((160, 256), 0)
    h_row = 2 * _div_small(rho2, 40, 160) + (rho2 & 1)
    w3 = wphi[...].astype(F32)
    wfd = jnp.concatenate([w3[d] for d in range(DH)], axis=1).astype(BF16)
    kk = _iota((D, D), 0)
    perm = (_iota((D, D), 1) == DH * (kk & (H - 1)) + (kk >> 5)).astype(BF16)
    wfh = _dot(wfd, perm, NN).astype(BF16)
    for blk in range(4):
        col = _iota((160, 256), 1) + (128 * blk - 160 * blk)
        t = _dot(eT, wfh[:, 128 * blk:128 * blk + 256], NN)
        bd_s[blk] = jnp.where((col >= DH * h_row) & (col < DH * h_row + DH), t, 0.0).astype(BF16)
    kvacc[...] = jnp.zeros_like(kvacc)

    def fold(dst, row0, col0):
        for blk in range(4):
            dst[pl.ds(row0 + 160 * blk, 160), :] = (
                _dot(bd_s[blk], wqkv[:, pl.ds(col0 + 128 * blk, 256)], NT) * LOG2E).astype(BF16)

    c_wq.wait()
    c_wv.start()
    for c in cx[:NS]:
        c.start()
    fold(wqT, 0, 0)
    c_wk.wait()
    fold(wkvT, 0, D)
    c_wv.wait()
    wkvT[D:2 * D, :] = wqkv[:, 2 * D:3 * D].T
    for st in range(NS):
        cx[st].wait()
    for c in cx[NS:]:
        c.start()

    def k_pass(st, rs):
        p_s[st] = _dot(wkvT[0:D, :], xn_s[rs, :], NT)
        yield
        for r in range(16):
            phi_s[st, pl.ds(80 * r, 80), :] = _hedgehog_pair(p_s[st, pl.ds(40 * r, 40), :])
        yield
        vT = _dot(wkvT[D:2 * D, :], xn_s[rs, :], NT).reshape(16, 40, SC)
        vx_s[st] = jnp.concatenate([vT, jnp.ones((16, 8, SC), F32)], axis=1).reshape(768, SC).astype(BF16)
        yield
        for sg in range(2):
            for c in range(5):
                p0, p1 = CH_PAIRS[c]
                m = 48 * (p1 - p0)
                r = _dot(vx_s[st, pl.ds(48 * (8 * sg + p0), m), :],
                         phi_s[st, pl.ds(640 * sg + 128 * c, 128), :], NT)
                kvacc[5 * sg + c, 0:m, :] += r
        yield

    def finalize_kv():
        for c in range(5):
            p0, p1 = CH_PAIRS[c]
            m = 48 * (p1 - p0)
            row = _iota((m, 128), 0)
            rp = _div_small(row, 48, 144)
            within = row - 48 * rp
            hh_row = jnp.where(within < 40, (within >= 20).astype(jnp.int32), (within >= 44).astype(jnp.int32))
            rho_c = _iota((m, 128), 1) + 128 * c
            cp = _div_small(rho_c, 80, 640) - p0
            ok = (cp == rp) & ((rho_c & 1) == hh_row)
            for sg in range(2):
                kvl[5 * sg + c, 0:m, :] = jnp.where(ok, kvacc[5 * sg + c, 0:m, :], 0.0).astype(BF16)
        kvacc[...] = jnp.zeros_like(kvacc)

    def attn_out(st, xn, resid):
        p_s[st] = _dot(wqT[...], xn, NT)
        yield
        for r in range(16):
            phi_s[st, pl.ds(80 * r, 80), :] = _hedgehog_pair(p_s[st, pl.ds(40 * r, 40), :])
        yield
        lo = _iota((8, SC), 0) < 4
        rows = []
        for sg in range(2):
            acc = [None] * 8
            for c in range(5):
                p0, p1 = CH_PAIRS[c]
                m = 48 * (p1 - p0)
                r = _dot(kvl[5 * sg + c, 0:m, :], phi_s[st, pl.ds(640 * sg + 128 * c, 128), :], NN)
                for j, p in enumerate(range(p0, p1)):
                    piece = r[48 * j:48 * j + 48]
                    acc[p] = piece if acc[p] is None else acc[p] + piece
            for p in range(8):
                a = acc[p]
                rmid = 1.0 / (a[40:48] + 1e-6)
                rrot = pltpu.roll(rmid, 4, 0)
                r0 = jnp.where(lo, rmid, rrot)
                r1 = jnp.where(lo, rrot, rmid)
                rows += [a[0:8] * r0, a[8:16] * r0, a[16:24] * rmid, a[24:32] * r1, a[32:40] * r1]
        oT = jnp.concatenate(rows, axis=0)
        o = oT.T.astype(BF16)
        x1_s[st] = resid() + _dot(o, wo[...], NN)
        yield

    def ffn(st, emit):
        for j in range(0, SC, LNB):
            xh_s[st, pl.ds(j, LNB), :] = _layernorm(x1_s[st, pl.ds(j, LNB), :], 0.5)
        yield
        xh = xh_s[st]
        for n0 in range(0, F, 256):
            n1 = min(F, n0 + 256)
            hh = _dot(xh, w1[n0:n1, :], NT)
            h_s[st, :, n0:n1] = (hh * jnp.tanh(hh) + hh).astype(BF16)
        for n0 in range(0, D, NB2):
            n1 = min(D, n0 + NB2)
            emit(n0, n1, x1_s[st, :, n0:n1] + _dot(h_s[st], w2[:, n0:n1], NN))
        yield

    def rows_of(i, st):
        return pl.ds(pl.multiple_of((NS * i + st) * SC, SC), SC)

    def s_update(i, st):
        rs = rows_of(i, st)
        yield from attn_out(st, xn_s[rs, :], lambda: xres[rs, :].astype(F32))
        def emit(n0, n1, x2):
            xres[rs, n0:n1] = x2.astype(BF16)
        yield from ffn(st, emit)

    def s_norm(i):
        for st in range(NS):
            for j in range(0, SC, LNB):
                rs = pl.ds(pl.multiple_of((NS * i + st) * SC + j, LNB), LNB)
                xn_s[rs, :] = _layernorm(xres[rs, :].astype(F32), 1.0)
            yield

    NIT = NCH // NS

    def layer(l, carry):
        _interleave([s_norm(0)], "0" * NS)

        def loop_stats(i, c):
            @pl.when(jnp.logical_and(l == 0, i < NIT - 1))
            def _():
                for st in range(NS):
                    pltpu.make_async_copy(x_hbm.at[pl.ds(0, SC)], xres.at[pl.ds(0, SC)],
                                          sem_x.at[NS * (i + 1) + st]).wait()

            @pl.when(jnp.logical_and(l == 0, i == 1))
            def _():
                c_wo.start()
                c_w1.start()
                c_w2.start()
            nxt = jnp.where(i == NIT - 1, 0, i + 1)
            _interleave([k_pass(st, rows_of(i, st)) for st in range(NS)] + [s_norm(nxt)], STAT_ORDER)
            return c
        lax.fori_loop(0, NIT, loop_stats, 0)

        @pl.when(l == 0)
        def _():
            c_wo.wait()
            c_w1.wait()
            c_w2.wait()
        finalize_kv()

        def loop_update(i, c):
            _interleave([s_update(i, st) for st in range(NS)], UPD_ORDER)

            @pl.when(l == 1)
            def _():
                rs = pl.ds(pl.multiple_of(NS * i * SC, NS * SC), NS * SC)
                pltpu.make_async_copy(xres.at[rs], out_hbm.at[rs], sem_o.at[i]).start()
            return c
        lax.fori_loop(0, NCH // NS, loop_update, 0)
        return carry
    lax.fori_loop(0, 2, layer, 0)
    for i in range(NCH // NS):
        rs = pl.ds(i * NS * SC, NS * SC)
        pltpu.make_async_copy(xres.at[rs], out_hbm.at[rs], sem_o.at[i]).wait()


@jax.jit
def pallas_interleave_layers__linear_kernel_hedgehog__dense_activation_silu__prompt_kernel(A_x, A_wqkv, A_w_phi, A_wo, B_x, B_w1, B_w2):
    any_spec = pl.BlockSpec(memory_space=pltpu.HBM)
    out = pl.pallas_call(
        kernel,
        in_specs=[any_spec] * 6,
        out_specs=any_spec,
        out_shape=jax.ShapeDtypeStruct((S, D), BF16),
        scratch_shapes=[
            pltpu.VMEM((S, D), BF16),
            pltpu.VMEM((D, 3 * D), BF16),
            pltpu.VMEM((DH, DH, H), BF16),
            pltpu.VMEM((D, D), BF16),
            pltpu.VMEM((F, D), BF16),
            pltpu.VMEM((F, D), BF16),
            pltpu.VMEM((D, D), BF16),
            pltpu.VMEM((2 * D, D), BF16),
            pltpu.VMEM((S, D), BF16),
            pltpu.VMEM((10, 144, 128), F32),
            pltpu.VMEM((10, 144, 128), BF16),
            pltpu.VMEM((NS, SC, F), BF16),
            pltpu.VMEM((NS, 1280, SC), BF16),
            pltpu.VMEM((NS, 768, SC), BF16),
            pltpu.VMEM((NS, D, SC), F32),
            pltpu.VMEM((NS, SC, D), F32),
            pltpu.VMEM((4, 160, 256), BF16),
            pltpu.VMEM((NS, SC, D), BF16),
            pltpu.SemaphoreType.DMA((NCH,)),
            pltpu.SemaphoreType.DMA((7,)),
            pltpu.SemaphoreType.DMA((NCH,)),
        ],
        compiler_params=pltpu.CompilerParams(vmem_limit_bytes=100 * 1024 * 1024, flags=FLAGS),
    )(A_x.reshape(S, D), A_wqkv, A_w_phi.transpose(1, 2, 0), A_wo, B_w1.T, B_w2)
    return out.reshape(1, S, D)
```

```python
import functools
import jax
import jax.numpy as jnp
from jax import lax
import jax.experimental.pallas as pl
import jax.experimental.pallas.tpu as pltpu

S, D, H, DH, F = 2048, 640, 32, 20, 1728
SC = 256
NCH = S // SC
NS = 2
STAT_ORDER = "0122010011"
UPD_ORDER = "010101010101"
FLAGS = {"XLA_TPU_EVENLY_DISTRIBUTE_CRITICAL_NODES": True}
LNB = 16
MB = 80
MV = 320
NBO = 128
FM = F // 128 * 128
NB1 = 256
NB2 = 128
LOG2E = 1.4426950408889634
F32, BF16 = jnp.float32, jnp.bfloat16

NT = (((1,), (1,)), ((), ()))
NN = (((1,), (0,)), ((), ()))

WIN = [min(80 * r, 1280 - 128) for r in range(16)]


def _dot(a, b, dims):
    return lax.dot_general(a, b, dims, preferred_element_type=F32)


def _iota(shape, dim):
    return lax.broadcasted_iota(jnp.int32, shape, dim)


def _div_small(v, d, vmax):
    out = jnp.zeros_like(v)
    for t in range(d, vmax, d):
        out = out + (v >= t).astype(jnp.int32)
    return out


def _layernorm(x, scale):
    m = jnp.mean(x, axis=-1, keepdims=True)
    xc = x - m
    v = jnp.mean(xc * xc, axis=-1, keepdims=True)
    return (xc * (lax.rsqrt(v + 1e-5) * scale)).astype(BF16)


def _pair_reduce(y, op):
    y = op(y, pltpu.roll(y, 4, 0))
    return op(y, pltpu.roll(y, 2, 0))


def _hedgehog_pair(p):
    ps = [p[8 * i:8 * i + 8] for i in range(5)]
    mx = _pair_reduce(functools.reduce(jnp.maximum, ps), jnp.maximum)
    mn = _pair_reduce(functools.reduce(jnp.minimum, ps), jnp.minimum)
    ep = [jnp.exp2(q - mx) for q in ps]
    em = [jnp.exp2(mn - q) for q in ps]
    rp = 1.0 / _pair_reduce(functools.reduce(jnp.add, ep), jnp.add)
    rm = 1.0 / _pair_reduce(functools.reduce(jnp.add, em), jnp.add)
    return jnp.concatenate([e * rp for e in ep] + [e * rm for e in em], axis=0).astype(BF16)


def _interleave(gens, order):
    gens = list(gens)
    for ch in order:
        next(gens[int(ch)])
    done = object()
    for g in gens:
        assert next(g, done) is done


def kernel(x_hbm, wqkv_hbm, wphi_hbm, wo_hbm, w1_hbm, w2_hbm, out_hbm,
           xres, wqkv, wphi, wo, w1, w2, wqT, wkvT, xn_s, kvacc, kvl,
           h_s, phi_s, vx_s, p_s, x1_s, bd_s, xh_s, sem_x, sem_w, sem_o):
    cx = [pltpu.make_async_copy(x_hbm.at[pl.ds(i * NS * SC, NS * SC)], xres.at[pl.ds(i * NS * SC, NS * SC)],
                                sem_x.at[i]) for i in range(NCH // NS)]
    cols = [pl.ds(j * D, D) for j in range(3)]
    cw = [pltpu.make_async_copy(a, b, sem_w.at[i]) for i, (a, b) in enumerate(
        [(wphi_hbm, wphi), (wo_hbm, wo), (w1_hbm, w1), (w2_hbm, w2)]
        + [(wqkv_hbm.at[:, c], wqkv.at[:, c]) for c in cols])]
    c_phi, c_wo, c_w1, c_w2, c_wq, c_wk, c_wv = cw
    c_phi.start()
    c_wq.start()
    c_wk.start()
    cx[0].start()

    c_phi.wait()
    rho = _iota((160, 128), 0)
    f_of = (rho - 40 * _div_small(rho, 40, 160)) >> 1
    eT = (f_of == _iota((160, 128), 1)).astype(BF16)[:, :DH]
    rho2 = _iota((160, 256), 0)
    h_row = 2 * _div_small(rho2, 40, 160) + (rho2 & 1)
    w3 = wphi[...].astype(F32)
    wfd = jnp.concatenate([w3[d] for d in range(DH)], axis=1).astype(BF16)
    kk = _iota((D, D), 0)
    perm = (_iota((D, D), 1) == DH * (kk & (H - 1)) + (kk >> 5)).astype(BF16)
    wfh = _dot(wfd, perm, NN).astype(BF16)
    for blk in range(4):
        col = _iota((160, 256), 1) + (128 * blk - 160 * blk)
        t = _dot(eT, wfh[:, 128 * blk:128 * blk + 256], NN)
        bd_s[blk] = jnp.where((col >= DH * h_row) & (col < DH * h_row + DH), t, 0.0).astype(BF16)
    kvacc[...] = jnp.zeros_like(kvacc)

    def fold(dst, row0, col0):
        for blk in range(4):
            dst[pl.ds(row0 + 160 * blk, 160), :] = (
                _dot(bd_s[blk], wqkv[:, pl.ds(col0 + 128 * blk, 256)], NT) * LOG2E).astype(BF16)

    c_wq.wait()
    c_wv.start()
    cx[1].start()
    fold(wqT, 0, 0)
    c_wk.wait()
    cx[0].wait()
    fold(wkvT, 0, D)
    for j in range(0, NS * SC, LNB):
        xn_s[pl.ds(j, LNB), :] = _layernorm(xres[pl.ds(j, LNB), :].astype(F32), 1.0)
    c_wv.wait()
    for c in cx[2:]:
        c.start()
    wkvT[D:2 * D, :] = wqkv[:, 2 * D:3 * D].T

    def k_pass(st, rs):
        xn = xn_s[rs, :]
        for m0 in range(0, D, MB):
            p_s[st, m0:m0 + MB, :] = _dot(wkvT[m0:m0 + MB, :], xn, NT)
        yield
        for r in range(16):
            phi_s[st, pl.ds(80 * r, 80), :] = _hedgehog_pair(p_s[st, pl.ds(40 * r, 40), :])
        yield
        for m0 in range(0, D, MV):
            n = MV // 40
            vT = _dot(wkvT[D + m0:D + m0 + MV, :], xn, NT).reshape(n, 40, SC)
            vx_s[st, pl.ds(48 * (m0 // 40), 48 * n), :] = jnp.concatenate(
                [vT, jnp.ones((n, 8, SC), F32)], axis=1).reshape(48 * n, SC).astype(BF16)
        yield
        for r in range(16):
            kvacc[r] += _dot(vx_s[st, pl.ds(48 * r, 48), :], phi_s[st, pl.ds(WIN[r], 128), :], NT)
        yield

    def finalize_kv():
        row = _iota((48, 128), 0)
        col = _iota((48, 128), 1)
        hh_row = jnp.where(row < 40, (row >= 20).astype(jnp.int32), (row >= 44).astype(jnp.int32))
        same_head = (col & 1) == hh_row
        for r in range(16):
            off = 80 * r - WIN[r]
            ok = same_head & (col >= off) & (col < off + 80)
            kvl[r] = jnp.where(ok, kvacc[r], 0.0).astype(BF16)
        kvacc[...] = jnp.zeros_like(kvacc)

    def attn_out(st, xn, resid):
        for m0 in range(0, D, MB):
            p_s[st, m0:m0 + MB, :] = _dot(wqT[m0:m0 + MB, :], xn, NT)
        yield
        for r in range(16):
            phi_s[st, pl.ds(80 * r, 80), :] = _hedgehog_pair(p_s[st, pl.ds(40 * r, 40), :])
        yield
        lo = _iota((8, SC), 0) < 4
        rows = []
        for r in range(16):
            a = _dot(kvl[r], phi_s[st, pl.ds(WIN[r], 128), :], NN)
            rmid = 1.0 / (a[40:48] + 1e-6)
            rrot = pltpu.roll(rmid, 4, 0)
            r0 = jnp.where(lo, rmid, rrot)
            r1 = jnp.where(lo, rrot, rmid)
            rows += [a[0:8] * r0, a[8:16] * r0, a[16:24] * rmid, a[24:32] * r1, a[32:40] * r1]
        oT = jnp.concatenate(rows, axis=0)
        xh_s[st] = oT.T.astype(BF16)
        yield
        for n0 in range(0, D, NBO):
            x1_s[st, :, n0:n0 + NBO] = resid(n0, n0 + NBO) + _dot(xh_s[st], wo[:, n0:n0 + NBO], NN)
        yield

    def ffn(st, emit, done):
        for j in range(0, SC, LNB):
            xh_s[st, pl.ds(j, LNB), :] = _layernorm(x1_s[st, pl.ds(j, LNB), :], 0.5)
        yield
        xh = xh_s[st]
        for n0 in range(0, FM, NB1):
            n1 = min(FM, n0 + NB1)
            hh = _dot(xh, w1[n0:n1, :], NT)
            h_s[st, :, n0:n1] = (hh * jnp.tanh(hh) + hh).astype(BF16)
        ht = _dot(w1[FM:F, :], xh, NT)
        h_s[st, :, FM:F] = (ht * jnp.tanh(ht) + ht).T.astype(BF16)
        for n0 in range(0, D, NB2):
            n1 = min(D, n0 + NB2)
            emit(n0, n1, x1_s[st, :, n0:n1] + _dot(h_s[st], w2[:, n0:n1], NN))
        done()
        yield

    def rows_of(i, st):
        return pl.ds(pl.multiple_of((NS * i + st) * SC, SC), SC)

    def out_copy(rs):
        return pltpu.make_async_copy(xres.at[rs], out_hbm.at[rs], sem_o)

    def s_update(i, st):
        rs = rows_of(i, st)
        yield from attn_out(st, xn_s[rs, :], lambda n0, n1: xres[rs, n0:n1].astype(F32))
        def emit(n0, n1, x2):
            xres[rs, n0:n1] = x2.astype(BF16)
        yield from ffn(st, emit, out_copy(rs).start)

    def s_norm(i):
        for st in range(NS):
            for j in range(0, SC, LNB):
                rs = pl.ds(pl.multiple_of((NS * i + st) * SC + j, LNB), LNB)
                xn_s[rs, :] = _layernorm(xres[rs, :].astype(F32), 1.0)
            yield

    NIT = NCH // NS

    def layer(l, carry):
        @pl.when(l == 1)
        def _():
            for st in range(NS):
                xn_s[pl.ds(st * SC, SC), :] = _layernorm(xres[pl.ds(st * SC, SC), :].astype(F32), 1.0)

        def loop_stats(i, c):
            @pl.when(jnp.logical_and(l == 0, i < NIT - 1))
            def _():
                rows = pl.ds(pl.multiple_of((i + 1) * NS * SC, NS * SC), NS * SC)
                pltpu.make_async_copy(x_hbm.at[rows], xres.at[rows], sem_x.at[i + 1]).wait()

            @pl.when(jnp.logical_and(l == 0, i == 1))
            def _():
                c_wo.start()
                c_w1.start()
                c_w2.start()
            nxt = jnp.where(i == NIT - 1, 0, i + 1)
            _interleave([k_pass(st, rows_of(i, st)) for st in range(NS)] + [s_norm(nxt)], STAT_ORDER)
            return c
        lax.fori_loop(0, NIT, loop_stats, 0)

        @pl.when(l == 0)
        def _():
            c_wo.wait()
            c_w1.wait()
            c_w2.wait()

        @pl.when(l == 1)
        def _():
            pltpu.make_async_copy(xres, out_hbm, sem_o).wait()
        finalize_kv()

        def loop_update(i, c):
            _interleave([s_update(i, st) for st in range(NS)], UPD_ORDER)

            return c
        lax.fori_loop(0, NCH // NS, loop_update, 0)
        return carry
    lax.fori_loop(0, 2, layer, 0)
    pltpu.make_async_copy(xres, out_hbm, sem_o).wait()


@jax.jit
def pallas_interleave_layers__linear_kernel_hedgehog__dense_activation_silu__prompt_kernel(A_x, A_wqkv, A_w_phi, A_wo, B_x, B_w1, B_w2):
    del B_x
    any_spec = pl.BlockSpec(memory_space=pltpu.HBM)
    out = pl.pallas_call(
        kernel,
        in_specs=[any_spec] * 6,
        out_specs=any_spec,
        out_shape=jax.ShapeDtypeStruct((S, D), BF16),
        scratch_shapes=[
            pltpu.VMEM((S, D), BF16),
            pltpu.VMEM((D, 3 * D), BF16),
            pltpu.VMEM((DH, DH, H), BF16),
            pltpu.VMEM((D, D), BF16),
            pltpu.VMEM((F, D), BF16),
            pltpu.VMEM((F, D), BF16),
            pltpu.VMEM((D, D), BF16),
            pltpu.VMEM((2 * D, D), BF16),
            pltpu.VMEM((S, D), BF16),
            pltpu.VMEM((16, 48, 128), F32),
            pltpu.VMEM((16, 48, 128), BF16),
            pltpu.VMEM((NS, SC, F), BF16),
            pltpu.VMEM((NS, 1280, SC), BF16),
            pltpu.VMEM((NS, 768, SC), BF16),
            pltpu.VMEM((NS, D, SC), F32),
            pltpu.VMEM((NS, SC, D), F32),
            pltpu.VMEM((4, 160, 256), BF16),
            pltpu.VMEM((NS, SC, D), BF16),
            pltpu.SemaphoreType.DMA((NCH // NS,)),
            pltpu.SemaphoreType.DMA((7,)),
            pltpu.SemaphoreType.DMA(()),
        ],
        compiler_params=pltpu.CompilerParams(vmem_limit_bytes=100 * 1024 * 1024, flags=FLAGS),
    )(A_x.reshape(S, D), A_wqkv, A_w_phi.transpose(1, 2, 0), A_wo, B_w1.T, B_w2)
    return out.reshape(1, S, D)
```
